```python
import os as _os
_os.environ.setdefault("JAX_PLATFORMS", "cpu")
import jax
import jax.numpy as jnp

def _softmax(x, axis=-1):
    return jax.nn.softmax(x, axis=axis)
def _gelu(x):
    return jax.nn.gelu(x, approximate=True)
def _silu(x):
    return jax.nn.silu(x)
def _sigmoid(x):
    return jax.nn.sigmoid(x)
def _layernorm(x, axis=-1, eps=1e-5):
    m = jnp.mean(x, axis=axis, keepdims=True)
    v = jnp.var(x, axis=axis, keepdims=True)
    return (x - m) / jnp.sqrt(v + eps)
def _scatter_add(tgt, idx, src, axis=0):
    return tgt.at[idx].add(src)
def _segment_sum(src, seg, n):
    return jax.ops.segment_sum(src, seg, n)
class _Rng:
    def __init__(self, key):
        self._k = key
    def _next(self):
        self._k, sub = jax.random.split(self._k)
        return sub
    def normal(self, shape):
        return jax.random.normal(self._next(), shape, dtype=jnp.bfloat16)
    def randint(self, lo, hi, shape):
        return jax.random.randint(self._next(), shape, lo, hi, dtype=jnp.int32)
    def uniform(self, shape, lo=0.0, hi=1.0):
        return jax.random.uniform(self._next(), shape, jnp.bfloat16, lo, hi)
    def permutation(self, n):
        return jax.random.permutation(self._next(), n)


kernel_name = 'sequential_preLN__sliding_block__mixer_channel_mlp__prompt'

def setup_inputs():
    _rng = _Rng(jax.random.key(int.from_bytes(__import__("os").urandom(4), "little")))
    _w = (lambda a: (lambda t: t.astype(jnp.bfloat16) if jnp.issubdtype(t.dtype, jnp.floating) else t)(jnp.asarray(a)))
    def _A_setup():
        B, S, D = 1, 2048, 1024
        return {
            "x": _w((lambda *s: _rng.normal(s) * 0.05)(B, S, D)),
            "wqkv": _w((lambda *s: _rng.normal(s) * 0.05)(D, 3 * D)),
            "wo": _w((lambda *s: _rng.normal(s) * 0.05)(D, D)),
        }
    _A_in = _A_setup()

    def _B_setup():
        B, S, D, F = 1, 2048, 1024, 3584
        return {
            "x": _w((lambda *s: _rng.normal(s) * 0.05)(B, S, D)),
            "w1": _w((lambda *s: _rng.normal(s) * 0.8)(D, F) * (D ** -0.5)),
            "b1": _w((lambda *s: _rng.normal(s) * 0.8)(F)),
            "w2": _w((lambda *s: _rng.normal(s) * 0.8)(F, D) * (F ** -0.5)),
            "b2": _w((lambda *s: _rng.normal(s) * 0.05)(D)),
        }
    _B_in = _B_setup()

    return {
        "A_x": _A_in["x"],
        "A_wqkv": _A_in["wqkv"],
        "A_wo": _A_in["wo"],
        "B_x": _B_in["x"],
        "B_w1": _B_in["w1"],
        "B_b1": _B_in["b1"],
        "B_w2": _B_in["w2"],
        "B_b2": _B_in["b2"],
    }

def reference(A_x, A_wqkv, A_wo, B_x, B_w1, B_b1, B_w2, B_b2):
    def _A_ref(x, wqkv, wo):
        B, S, D = x.shape
        H = 32; Dh = D // H; W = 256
        qkv = (lambda x, *d: x.transpose(*d))((x @ wqkv).reshape(B, S, 3, H, Dh), 2, 0, 3, 1, 4)
        q, k, v = qkv[0], qkv[1], qkv[2]
        scores = jnp.einsum("bhqd,bhkd->bhqk", q, k) * (Dh ** -0.5)
        idx = jnp.arange(S)
        mask = (idx[:, None] - idx[None, :] >= 0) & (idx[:, None] - idx[None, :] < W)
        scores = jnp.where(mask[None, None], scores, -1e9)
        p = _softmax(scores, axis=-1)
        o = jnp.einsum("bhqk,bhkd->bhqd", p, v)
        return (lambda x, *d: x.transpose(*d))(o, 0, 2, 1, 3).reshape(B, S, D) @ wo

    def _B_ref(x, w1, b1, w2, b2):
        y = _layernorm(x, axis=-1)
        h = _gelu(jnp.einsum("bsd,df->bsf", y, w1) + b1)
        return jnp.einsum("bsf,fd->bsd", h, w2) + b2

    x = A_x
    h = x + _A_ref(_layernorm(x, axis=-1), A_wqkv, A_wo)
    h2 = h + _B_ref(_layernorm(h, axis=-1), B_w1, B_b1, B_w2, B_b2)
    return h2
```

```python
import functools

import numpy as np
import jax
import jax.numpy as jnp
from jax import lax
import jax.experimental.pallas as pl
import jax.experimental.pallas.tpu as pltpu

H, W = 32, 256
BM = 256
FLAGS = None
ONLY = '0AB'
FENCES = '12'
DELAY, TAIL, FRAC, NPRE, GELU_Y, LAG = 10, 10, 0.4, 7, 8, 0
TIE_MOD = 7
ORDER = 1
F2 = 0.05
OSPLIT = 0.33
PAD = 16
HEAD = 14
HSTEPS = 8
ROWS0 = 64
QT = True
TIE0 = False
F1 = 0.1
SCHED = 0
EPS = 1e-5
LOG2E = 1.4426950408889634
F32, BF16, U32 = jnp.float32, jnp.bfloat16, jnp.uint32
HDT = F32


def _merge(*streams):
    def gen():
        state = [[g, max(n, 1), 0] for g, n in streams]
        while state:
            s = min(state, key=lambda e: (e[2] + 0.5) / e[1])
            try:
                next(s[0])
                s[2] += 1
                yield
            except StopIteration:
                state.remove(s)
    return gen(), sum(n for _, n in streams)


def _chain(*streams):
    def gen():
        for g, _ in streams:
            yield from g
    return gen(), sum(n for _, n in streams)


def _take(stream, n):
    return (next(stream[0]) for _ in range(n)), n


def _run(*streams):
    for _ in _merge(*streams)[0]:
        pass


def _cat(xs, axis):
    return xs[0] if len(xs) == 1 else jnp.concatenate(xs, axis=axis)


def _dot(a, b):
    return jnp.dot(a, b, preferred_element_type=F32)


def _dot_nt(a, b):
    return lax.dot_general(a, b, (((1,), (1,)), ((), ())), preferred_element_type=F32)


class _Slabs:
    def __init__(self, ref, rows, base=0):
        self.ref, self.rows, self.base, self.step = ref, rows, base, rows + PAD

    def window(self, first, count):
        start = self.base + first * self.step
        if isinstance(start, int):
            return _Slabs(self.ref, self.rows, start)
        return _Slabs(self.ref.at[pl.ds(pl.multiple_of(start, 16), count * self.step)], self.rows)

    def words(self, idx, r0=0, r1=None):
        start = self.base + idx * self.step
        return self.ref.bitcast(U32)[(start + r0) // 2:(start + (r1 or self.rows)) // 2, :]

    def load(self, idx, r0=0, r1=None):
        return pltpu.bitcast(self.words(idx, r0, r1), BF16)

    def store(self, idx, r0, v):
        start = self.base + idx * self.step + r0
        self.ref[start:start + v.shape[0], :] = v.astype(BF16)

    def all(self, idx):
        return self.ref.at[pl.ds(self.base + idx * self.step, self.rows)]


class _Order:
    def __init__(self, never=None):
        self.never, self.results, self.pending = never, [], []

    def _tie(self, dep, v):
        head = jnp.where(self.never, dep, v[0:8, 0:128])
        head = _cat([head] + ([v[0:8, 128:]] if v.shape[1] > 128 else []), 1)
        return _cat([head] + ([v[8:]] if v.shape[0] > 8 else []), 0)

    def after_matmul(self, v):
        if self.never is None or len(self.results) <= LAG:
            return v
        return self._tie(self.results[-1 - LAG], v)

    def before_matmul(self, v):
        if self.never is not None:
            self.pending.append(v[0:8, 0:128])

    def matmul(self, words, rhs, dot=_dot):
        for dep in self.pending:
            words = self._tie(pltpu.bitcast(dep, U32), words)
        self.pending = []
        r = dot(pltpu.bitcast(words, BF16), rhs)
        self.results.append(r[0:8, 0:128])
        return r


_FLIP = (1, 0, 1, 1, 0, 0, 1)


def _add(p, q, sign=1):
    if isinstance(p, list):
        return [_add(a, b, sign) for a, b in zip(p, q)]
    return p + q if sign > 0 else p - q


def _operands(g, side, leaf=1, flip=0, base=0):
    if len(g) == leaf:
        yield base, flip, g
        return
    n = len(g) // 2
    x11, x12 = [r[:n] for r in g[:n]], [r[n:] for r in g[:n]]
    x21, x22 = [r[:n] for r in g[n:]], [r[n:] for r in g[n:]]
    if side == "a":
        terms = [(x21, x11, -1), (x11, x22, 1), (x12, x22, -1), (x21, x22, 1), (x22,), (x11,), (x11, x12, 1)]
    else:
        if flip:
            x11, x12, x21, x22 = x12, x11, x22, x21
        terms = [(x11, x12, 1), (x11, x22, 1), (x21, x22, 1), (x11,), (x21, x11, -1), (x12, x22, -1), (x22,)]
    for i, t in enumerate(terms):
        yield from _operands(t[0] if len(t) == 1 else _add(*t), side, leaf, flip ^ _FLIP[i], base * 7 + i)


def _products(f, level, flip=0, base=0):
    if level == 0:
        return (yield from f(base, flip))
    sub = lambda i: _products(f, level - 1, flip ^ _FLIP[i], base * 7 + i)
    m6 = yield from sub(0)
    m1 = yield from sub(1)
    c22 = _add(m6, m1)
    m7 = yield from sub(2)
    c11 = _add(m1, m7)
    m2 = yield from sub(3)
    c22 = _add(c22, m2, -1)
    m4 = yield from sub(4)
    c11 = _add(c11, m4)
    c21 = _add(m2, m4)
    m3 = yield from sub(5)
    c22 = _add(c22, m3)
    m5 = yield from sub(6)
    c11 = _add(c11, m5, -1)
    c12 = _add(m3, m5)
    if flip:
        c11, c12, c21, c22 = c12, c11, c22, c21
    return [a + b for a, b in zip(c11, c12)] + [a + b for a, b in zip(c21, c22)]


def _split(load, rows, cols, level, side, store, order=None, load_yields=0, row_groups=None):
    n = 2 ** level
    br, bc = rows // n, cols // n
    row_groups = range(0, br, 16) if row_groups is None else row_groups

    def gen():
        for r0 in row_groups:
            for t in range(bc // 128):
                g = []
                for a in range(n):
                    g.append([load(a * br + r0, b * bc + t * 128) for b in range(n)])
                    for _ in range(load_yields):
                        yield
                for p0, flip, g2 in _operands(g, side, 2):
                    for p, _, v in _operands(g2, side, 1, flip, p0):
                        store(p, t, r0, v[0][0], g2)
                        if p % TIE_MOD == 1 and order is not None:
                            order.before_matmul(v[0][0])
                    yield
    return gen(), len(row_groups) * bc // 128 * (7 ** (level - 1) + n * load_yields)


def _matmul(product, level, finish, steps=None):
    def gen():
        grid = yield from _products(product, level)
        br, bc = grid[0][0].shape
        finish({(i * br, j * bc + t): blk[:, t:t + 128]
                for i, row in enumerate(grid) for j, blk in enumerate(row) for t in range(0, bc, 128)})
    return gen(), steps or 7 ** level


def _simple_product(a, kt, b, order):
    def product(p, flip):
        r = order.matmul(_cat([a.words(p * kt + t) for t in range(kt)], 1), b.load(p))
        yield
        return [[r]]
    return product


def _layernorm(x):
    xc = x - jnp.mean(x, axis=-1, keepdims=True)
    return xc * lax.rsqrt(jnp.mean(xc * xc, axis=-1, keepdims=True) + EPS)


def _gelu(x):
    c0 = float(np.sqrt(2.0 / np.pi))
    hx = 0.5 * x
    return hx + hx * jnp.tanh(x * (c0 + (c0 * 0.044715) * (x * x)))


def _butterfly(a, m1, m2):
    def sel(m, p, q):
        if p is None and q is None:
            return None
        z = jnp.zeros_like(q if p is None else p)
        return jnp.where(m, z if p is None else p, z if q is None else q)
    b = [sel(m1, a[0], a[1]), sel(m1, a[1], a[0]), sel(m1, a[2], a[3]), sel(m1, a[3], a[2])]
    return [sel(m2, b[0], b[2]), sel(m2, b[1], b[3]), sel(m2, b[2], b[0]), sel(m2, b[3], b[1])]


def _attention(q_s, k_prev, k_cur, vt_prev, vt_cur, p_s, o_s, order):
    groups = o_s.shape[1] // 128
    units = [(j, g) for g in range(groups) for j in range(BM // 128)]

    def lanes(rows):
        return lax.broadcasted_iota(jnp.int32, (rows, 128), 1)
    tri = lax.broadcasted_iota(jnp.int32, (32, 128), 0) > (lanes(32) & 31)
    blk16, blk8, blk32 = lanes(16) >> 5, lanes(8) >> 5, lanes(32) >> 5
    sums = [[] for _ in units]
    pair, col = 2 * lax.broadcasted_iota(jnp.int32, (16, 128), 0), lanes(16) & 31
    tri_words = pltpu.bitcast(jnp.where(pair > col, 0xFFFF, 0) | jnp.where(pair + 1 > col, -0x10000, 0), U32)

    def lowest(j, t):
        return max(t, 8 - 4 * j) if k_prev is None else t

    def keys(g, a, b):
        return _cat(([k_prev.words(g, a, min(b, BM))] if a < BM else [])
                    + ([k_cur.words(g, max(a, BM) - BM, b - BM)] if b > BM else []), 0)

    def scores(u):
        j, g = units[u]
        for t in range(4):
            if True:
                q = [q_s.words(j * groups + g, 32 * h, 32 * h + 32) for h in range(4)]
                qd = pltpu.bitcast(_cat([jnp.where(blk16 == (h ^ t), q[h], jnp.zeros_like(q[h])) for h in range(4)], 0), BF16)
            else:
                q = q_s.words(j * groups + g, 32 * t, 32 * t + 32)
                qd = pltpu.bitcast(_cat([jnp.where(blk16 == (c ^ t), q, jnp.zeros_like(q)) for c in range(4)], 0), BF16)
            lo = lowest(j, t)
            for part, blocks in enumerate(([a for a in range(lo, t + 9) if not 4 <= a < 8], list(range(max(lo, 4), 8)))):
                if not blocks:
                    yield
                    continue
                kk = _cat([keys(g, j * 128 + 32 * a, j * 128 + 32 * a + 32) for a in blocks], 0)
                n = 2 if len(blocks) > 1 else 1
                step = kk.shape[0] // n
                s = _cat([order.matmul(kk[c * step:(c + 1) * step], qd, _dot if QT else _dot_nt) for c in range(n)], 0)
                s = [s[r:r + 32] for r in range(0, s.shape[0], 32)]
                if part == 0 and lo == t:
                    s = s[1:-1] + [jnp.where(tri, s[0], s[-1])]
                elif part == 0:
                    s[-1] = jnp.where(tri, -jnp.inf, s[-1])
                m = jnp.max(functools.reduce(jnp.maximum, s), axis=0, keepdims=True)
                e = [jnp.exp2(b - m) for b in s]
                sums[u].append((part, m, jnp.sum(functools.reduce(jnp.add, e), axis=0, keepdims=True)))
                for a, b in zip(blocks[len(blocks) - len(e):], e):
                    p_s.store((u % 3) * 4 + t, (a - t) * 32, b)
                yield

    def by_head(vals):
        v = [jnp.broadcast_to(x, (8, 128)) for x in vals]
        sub = lax.broadcasted_iota(jnp.int32, (8, 128), 0) ^ blk8
        return jnp.where((sub & 2) == 0, jnp.where((sub & 1) == 0, v[0], v[1]), jnp.where((sub & 1) == 0, v[2], v[3]))

    def values(u):
        j, g = units[u]
        acc, mid = [None] * 4, [None] * 4
        zero = jnp.zeros((16, 128), U32)
        for kt in range(3):
            if lowest(j, 0) >= 4 * kt + 4:
                yield
                yield
                continue
            ph = []
            for a in range(4 * kt, 4 * kt + 4):
                src = [None] * 4
                for t in range(4):
                    if lowest(j, t) <= a <= t + 8:
                        at = (8 if a == t else a - t) * 32
                        src[t] = p_s.words((u % 3) * 4 + t, at, at + 32)
                        if a == t or (a == t + 8 and lowest(j, t) == t):
                            src[t] = src[t] & (tri_words if a == t else ~tri_words)
                ph.append(_butterfly(src, (blk16 & 1) == 0, (blk16 & 2) == 0))
            yield
            vt = vt_prev if j + kt < 2 else vt_cur
            for h in range(4):
                p = _cat([zero if b[h] is None else b[h] for b in ph], 0)
                r = order.matmul(vt.words((j + kt) % 2 * groups + g, 32 * h, 32 * h + 32), pltpu.bitcast(p, BF16))
                if kt == 1:
                    mid[h] = r
                else:
                    acc[h] = r if acc[h] is None else acc[h] + r
            yield
        row = lambda v, h: jnp.broadcast_to(v[h:h + 1], (32, 128))
        m0, l0 = [by_head([x[n] for x in sums[u] if x[0] == 0]) for n in (1, 2)]
        if mid[0] is None:
            c0 = 1.0 / l0
            ot = _cat([acc[h] * row(c0, h) for h in range(4)], 0).T
        else:
            m1, l1 = [by_head([x[n] for x in sums[u] if x[0] == 1]) for n in (1, 2)]
            m = jnp.maximum(m0, m1)
            c0, c1 = jnp.exp2(m0 - m), jnp.exp2(m1 - m)
            inv = 1.0 / (c0 * l0 + c1 * l1)
            c0, c1 = c0 * inv, c1 * inv
            ot = _cat([acc[h] * row(c0, h) + mid[h] * row(c1, h) for h in range(4)], 0).T
        yield
        o = _butterfly([ot[32 * c:32 * c + 32] for c in range(4)], (blk32 & 1) == 0, (blk32 & 2) == 0)
        for t in range(4):
            o_s[j * 128 + 32 * t:j * 128 + 32 * t + 32, g * 128:(g + 1) * 128] = o[t]
        yield

    def gen():
        first_pass = (None for u in range(len(units)) for _ in scores(u))
        second_pass = (None for u in range(len(units)) for _ in values(u))
        for step in range(8 * len(units) + DELAY):
            next(first_pass, None)
            if step >= DELAY:
                next(second_pass, None)
            yield
        for _ in second_pass:
            pass
    return gen(), 8 * len(units) + DELAY


def _buffers(D, Fd):
    def rows(level, r, c):
        return 7 ** level * (c // 2 ** level // 128) * (r // 2 ** level + PAD)
    return dict(
        raw=4 * D // 128 * (D + PAD), w1=rows(2, D, Fd), w2=rows(2, Fd, D), gc=rows(2, BM, Fd),
        wa=rows(2, D, 4 * D),
        yc=rows(2, BM, D), oc=rows(2, BM, D), zc=rows(2, BM, D),
        q=2 * D // 128 * (128 + PAD), k=2 * D // 128 * (BM + PAD), vt=4 * D // 128 * (128 + PAD), p=12 * (288 + PAD))


def _kernel(x_hbm, wqkv_hbm, wo_hbm, w1_hbm, b1_hbm, w2_hbm, b2_hbm, out_hbm,
            h_s, o_s, b1_raw, b2_raw, b1_s, b2_s, x_s, raw1, raw2, out_s, bsem, xsem, qsem, wsem, osem, fsem, last_s, *pools):
    S, D = x_hbm.shape
    Fd = w1_hbm.shape[1]
    NB, NG = S // BM, D // 128
    NC = Fd // 512
    scale = float((D // H) ** -0.5 * LOG2E)
    buf = dict(zip(_buffers(D, Fd), pools))
    w1c, w2c = _Slabs(buf["w1"], D // 4), _Slabs(buf["w2"], Fd // 4)
    wac = _Slabs(buf["wa"], D // 4)
    raw = _Slabs(buf["raw"], D)
    yc, oc = _Slabs(buf["yc"], BM // 4), _Slabs(buf["oc"], BM // 4)
    y0, q_s, k_s, vt_s, p_s = [_Slabs(buf[n], r) for n, r in
                               (("zc", BM), ("q", 128), ("k", BM), ("vt", 128), ("p", 288))]
    zc, gc = _Slabs(buf["zc"], BM // 4), _Slabs(buf["gc"], BM // 4)

    b_copies = [pltpu.make_async_copy(b1_hbm, b1_raw, bsem.at[0]), pltpu.make_async_copy(b2_hbm, b2_raw, bsem.at[1])]
    x_copy = lambda b: pltpu.make_async_copy(
        x_hbm.at[pl.ds(b * BM, BM)], x_s.at[pl.ds(b * BM, BM)], xsem.at[b])

    def raw_copies(c):
        src, col = (wo_hbm, (c - 6) * 512) if isinstance(c, int) and c >= 6 else (wqkv_hbm, c * 512)
        dst = raw.window(c * 4, 4)
        return [pltpu.make_async_copy(src.at[:, pl.ds(pl.multiple_of(col + t * 128, 128), 128)],
                                      dst.all(t), qsem.at[c]) for t in range(4)]

    def next_rows(c):
        rows = [pl.ds(pl.multiple_of(BM + r + c * 16, 16), 16) for r in range(0, BM, BM // 4)]
        return [pltpu.make_async_copy(x_hbm.at[r], x_s.at[r], qsem.at[c]) for r in rows]

    w_copies = lambda c: [
        pltpu.make_async_copy(w1_hbm.at[:, pl.ds(c * 512, 512)], raw1.at[c % 2], wsem.at[c % 2]),
        pltpu.make_async_copy(w2_hbm.at[pl.ds(c * 512, 512)], raw2.at[c % 2], wsem.at[2 + c % 2])]
    out_copy = lambda b: pltpu.make_async_copy(
        out_s.at[b % 2], out_hbm.at[pl.ds(b * BM, BM)], osem.at[b % 2])

    def start(copies):
        for cp in copies:
            cp.start()

    def wait(copies):
        with jax.named_scope("wait"):
            for cp in copies:
                cp.wait()

    def fence(name):
        if name in FENCES:
            with jax.named_scope("fence"):
                pl.semaphore_signal(fsem, 1)
                pl.semaphore_wait(fsem, 1)

    def operand_store(slabs, tiles=1, base=0):
        return lambda p, t, r0, v, _: slabs.store(base + p * tiles + t, r0, v)

    def split_chunk(c, order):
        src = raw.window(c * 4, 4)
        return _split(lambda r0, c0: src.all(c0 // 128)[r0:r0 + 16, :].astype(F32),
                      D, 512, 2, "b", operand_store(wac.window(c * 49, 49)), order)

    def shifted(slabs, rows, most):
        return _Slabs(slabs.ref.at[pl.ds(pl.multiple_of(rows, 16), slabs.ref.shape[0] - most)], slabs.rows)

    def pieces(src):
        return lambda r0, c0: src[r0:r0 + 16, c0:c0 + 128].astype(F32)

    def normed_input(rows, times, dst, order, groups=range(0, BM // 4, 16)):
        done = {}

        def normalize(r):
            for r0 in range(r, BM, BM // 4):
                v = rows[r0:r0 + 16, :].astype(F32)
                for _ in range(times):
                    mean = jnp.mean(v, axis=-1, keepdims=True)
                    order.before_matmul(jnp.broadcast_to(mean, (16, 128)))
                    yield
                    v = v - mean
                    v = v * lax.rsqrt(jnp.mean(v * v, axis=-1, keepdims=True) + EPS)
                    order.before_matmul(v)
                    yield
                done[r0] = v
        return _chain(*[s for r in groups for s in (
            (normalize(r), 8 * times),
            _split(lambda r0, c0: done[r0][:, c0:c0 + 128], BM, D, 2, "a", operand_store(dst, 2), order, 0, [r]))])

    block = lambda ref, b: ref.at[pl.ds(pl.multiple_of(b * BM, BM), BM)]
    input_mlp = lambda b, order: normed_input(block(h_s, b), 2, zc, order)
    split_o = lambda order: _split(lambda r0, c0: o_s[r0:r0 + 16, c0:c0 + 128], BM, D, 2, "a",
                                   operand_store(oc, 2), order)

    def store_queries(dst, idx, v):
        if QT:
            blk = lax.broadcasted_iota(jnp.int32, (32, 128), 1) >> 5
            v = _cat(_butterfly([v[r:r + 32] for r in range(0, 128, 32)], (blk & 1) == 0, (blk & 2) == 0), 0).T
        dst.store(idx, 0, v)

    def out_proj(blk, order):
        rows = pl.ds(pl.multiple_of(blk * BM, BM), BM)
        x_rows, h_rows = x_s.at[rows], h_s.at[rows]

        def finish(c, tiles):
            for (r0, c0), v in tiles.items():
                at = slice(r0, r0 + v.shape[0]), slice(c * 512 + c0, c * 512 + c0 + 128)
                h_rows[at] = (x_rows[at].astype(F32) + v).astype(h_s.dtype)
        return _chain(*[_matmul(_simple_product(oc, 2, wac.window((6 + c) * 49, 0), order), 2,
                                functools.partial(finish, c)) for c in range(2)])

    if '0' in ONLY:
        first = raw_copies(0)
        start([x_copy(0)] + first[:2])
        wait([x_copy(0)])
        start(first[2:] + next_rows(0))
        y = _layernorm(x_s[0:BM, :].astype(F32))
        for g in range(NG):
            y0.store(g, 0, y[:, g * 128:(g + 1) * 128])

        start(raw_copies(1) + next_rows(1))

        def first_proj(src, tiles, store, order, rows=ROWS0):
            def gen():
                for t in range(tiles):
                    for r0 in range(0, BM, rows):
                        store(t, r0, order.matmul(_cat([y0.words(g, r0, r0 + rows) for g in range(NG)], 1), src.load(t)))
                        yield
            return gen(), BM // rows * tiles

        @pl.loop(0, 4)
        def _(c):
            order, last_s[0] = _Order(c < 0), c
            wait(raw_copies(c) + next_rows(c))
            start(raw_copies(c + 2))
            pl.when(c < 2)(lambda: start(next_rows(c + 2)))
            pl.when(c == 2)(lambda: start(raw_copies(6)))
            pl.when(c == 3)(lambda: start(raw_copies(7)))
            mul, dst = jnp.where(c < 2, scale, 1.0), k_s.window((c * 4 + NG) % (2 * NG), 4)
            _run(first_proj(raw.window(c * 4, 4), 4, lambda t, r0, r: dst.store(t, r0, r * mul), order),
                 _chain(split_chunk(c, order),
                        normed_input(x_s.at[pl.ds(pl.multiple_of(BM + c * 16, 16), BM - 48)], 1,
                                     shifted(yc, c * 16, 48), order, [0])))


        @pl.loop(0, 2)
        def _(c):
            order, parts = _Order(c < 0), []
            wait(raw_copies(4 + c))
            dst = vt_s.window(c * 4, NG + 4)

            def store(t, r0, r):
                parts.append(r)
                if (r0 + ROWS0) % 128 == 0:
                    dst.store(r0 // 128 * NG + t, 0, _cat(parts[-128 // ROWS0:], 0).T)
            _run(first_proj(raw.window((4 + c) * 4, 4), 4, store, order), split_chunk(4 + c, order))

        wait(raw_copies(6) + raw_copies(7))
        start(w_copies(0) + [x_copy(2)] + b_copies)
        order = _Order(last_s[0] < 0 if TIE0 else None)
        for g in range(NG):
            for j in range(2):
                store_queries(q_s, j * NG + g, k_s.all(NG + g)[j * 128:(j + 1) * 128, :].astype(F32))
        _run(_attention(q_s, None, k_s, None, vt_s, p_s, o_s, order),
             _chain(split_chunk(6, order), split_chunk(7, order)))

    @pl.loop(1, NB)
    def _(i):
        if 'A' not in ONLY: return
        order, last_s[0] = _Order(i < 0), i
        c = i - 1
        wait(w_copies(c))
        pl.when(i + 1 < NB)(lambda: wait([x_copy(i + 1)]))
        pl.when(i + 2 < NB)(lambda: start([x_copy(i + 2)]))
        pl.when(i < NC)(lambda: start(w_copies(i)))
        prep = _chain(
            _split(pieces(raw1.at[c % 2]), D, 512, 2, "b", operand_store(w1c.window(c * 49, 49)), order),
            _split(pieces(raw2.at[c % 2]), 512, D, 2, "b", operand_store(shifted(w2c, c * 128, Fd // 4 - 128), 2), order))
        k_new, vt_new = k_s.window(i % 2 * NG, NG), vt_s.window(i % 2 * 2 * NG, 2 * NG)

        def proj(c):
            def finish(tiles):
                for t in range(4):
                    v, g = _cat([tiles[k] for k in sorted(tiles) if k[1] == t * 128], 0), c % 2 * 4 + t
                    for j in range(2):
                        part = v[j * 128:(j + 1) * 128]
                        if c < 2:
                            store_queries(q_s, j * NG + g, part * scale)
                        elif c < 4:
                            k_new.store(g, j * 128, part)
                        else:
                            vt_new.store(j * NG + g, 0, part.T)
            return _matmul(_simple_product(yc, 2, wac.window(c * 49, 0), order), 2, finish)

        attention = lambda: _attention(
            q_s.window(jnp.minimum(i, 0), 2 * NG), k_s.window((i + 1) % 2 * NG, NG), k_s.window((i & 1) * NG, NG),
            vt_s.window((i + 1) % 2 * 2 * NG, 2 * NG), vt_s.window((i & 1) * 2 * NG, 2 * NG), p_s, o_s, _Order(i < 0))
        if SCHED == 0:
            parts = [proj(c) for c in [(4, 5, 0, 2, 1, 3), (4, 0, 2, 5, 1, 3), (0, 4, 1, 5, 2, 3), (4, 0, 2, 1, 3, 5)][ORDER]]
            main = _chain(*parts)
            n_o, late = int(main[1] * OSPLIT), _take(prep, int(prep[1] * F2))
            first = _take(prep, int(prep[1] * F1))
            _run(_take(main, n_o), _chain(split_o(order), first))
            _run(_take(main, main[1] - n_o - HEAD), _take(prep, prep[1] - first[1] - late[1]))
            fence('1')
            att = attention()
            _run((main[0], HEAD), _take(att, HSTEPS))
            _run(_take(att, att[1] - TAIL - HSTEPS))
            fence('2')
            wo = out_proj(i - 1, order)
            _run((att[0], TAIL), _take(wo, int(wo[1] * FRAC)))
            fence('3')
            _run((wo[0], wo[1] - int(wo[1] * FRAC)),
                 _chain(normed_input(block(x_s, jnp.minimum(i + 1, NB - 1)), 1, yc, order), (prep[0], late[1])))
        elif SCHED == 9:
            _run(attention())

    if '0' in ONLY:
        order = _Order(last_s[0] < 0)
        _run(split_o(None))
        wait(b_copies)
        b1_s[...] = jnp.broadcast_to(b1_raw[...].astype(F32).reshape(1, Fd), (8, Fd))
        b2_s[...] = jnp.broadcast_to(b2_raw[...].astype(F32).reshape(1, D), (8, D))
        _run(out_proj(NB - 1, order), input_mlp(0, order))

    @pl.loop(0, NB)
    def _(i):
        if 'B' not in ONLY: return
        order, hidden = _Order(i < 0), {}
        with jax.named_scope('waitout'):
            pl.when(i >= 2)(lambda: out_copy(i - 2).wait())

        def up(c):
            return _matmul(_simple_product(zc, 2, w1c.window(c * 49, 0), order), 2,
                           functools.partial(hidden.__setitem__, c))

        def activate(c):
            def load(r0, c0):
                bias = order.after_matmul(b1_s[:, c * 512 + c0:c * 512 + c0 + 128])
                return _gelu(hidden[c][(r0 // 64 * 64, c0)][r0 % 64:r0 % 64 + 16] + _cat([bias, bias], 0))
            return _split(load, BM, 512, 2, "a", operand_store(gc, NC, c), None, GELU_Y)

        def down(p, k0, k1):
            return order.matmul(_cat([gc.words(p * NC + t) for t in range(k0, k1)], 1),
                                _cat([w2c.load(p * 2 + t, k0 * 128, k1 * 128) for t in range(2)], 1))

        early = {}

        def product(p, flip):
            r = early.pop(p) + down(p, NC - 1, NC) if p in early else down(p, 0, NC)
            yield
            return [[r]]

        def head_start(n):
            for p in range(n):
                early[p] = down(p, 0, NC - 1)
                yield

        def finish(tiles):
            h_rows, dst = h_s.at[pl.ds(pl.multiple_of(i * BM, BM), BM)], out_s.at[i % 2]
            for (r0, c0), v in tiles.items():
                at = slice(r0, r0 + v.shape[0]), slice(c0, c0 + 128)
                dst[at] = (h_rows[at].astype(F32) + (v + _cat([b2_s[:, c0:c0 + 128]] * (v.shape[0] // 8), 0))).astype(out_s.dtype)

        _run(up(0))
        for c in range(1, NC):
            _run(up(c), activate(c - 1))
        _run((head_start(NPRE), NPRE), activate(NC - 1))
        _run(_matmul(product, 2, finish), input_mlp(jnp.minimum(i + 1, NB - 1), order))
        out_copy(i).start()

    if ONLY in 'A0':
        for bb in range(2):
            out_s[bb] = (o_s[...] + h_s[0:BM]).astype(BF16)
            for n_, sl_ in enumerate((w1c, w2c, wac, yc, _Slabs(zc.ref, 128))):
                out_s[bb, 0:128, n_ * 128:(n_ + 1) * 128] = sl_.window(last_s[0], 1).load(0, 0, 128) if sl_.rows >= 128 else _cat([sl_.window(last_s[0], 1).load(0)] * 2, 0)
            out_copy(bb).start()
    wait([out_copy(NB - 2), out_copy(NB - 1)])


def pallas_sequential_preLN__sliding_block__mixer_channel_mlp__prompt_kernel(
        A_x, A_wqkv, A_wo, B_x, B_w1, B_b1, B_w2, B_b2):
    B, S, D = A_x.shape
    Fd = B_w1.shape[1]
    dma = pltpu.SemaphoreType.DMA
    out = pl.pallas_call(
        _kernel,
        in_specs=[pl.BlockSpec(memory_space=pl.ANY)] * 7,
        out_specs=pl.BlockSpec(memory_space=pl.ANY),
        out_shape=jax.ShapeDtypeStruct((S, D), A_x.dtype),
        scratch_shapes=[
            pltpu.VMEM((S, D), HDT), pltpu.VMEM((BM, D), F32),
            pltpu.VMEM((Fd,), B_b1.dtype), pltpu.VMEM((D,), B_b2.dtype), pltpu.VMEM((8, Fd), F32), pltpu.VMEM((8, D), F32),
            pltpu.VMEM((S, D), BF16), pltpu.VMEM((2, D, 512), BF16), pltpu.VMEM((2, 512, D), BF16), pltpu.VMEM((2, BM, D), A_x.dtype),
            dma((2,)), dma((S // BM,)), dma((8,)), dma((4,)), dma((2,)), pltpu.SemaphoreType.REGULAR,
            pltpu.SMEM((1,), jnp.int32),
            *[pltpu.VMEM((n, 128), BF16) for n in _buffers(D, Fd).values()]],
        compiler_params=pltpu.CompilerParams(vmem_limit_bytes=127 << 20, flags=FLAGS),
        name="fused",
    )(A_x.reshape(S, D), A_wqkv, A_wo, B_w1, B_b1, B_w2, B_b2)
    return out.reshape(B, S, D)
```

```python
import functools

import numpy as np
import jax
import jax.numpy as jnp
from jax import lax
import jax.experimental.pallas as pl
import jax.experimental.pallas.tpu as pltpu

HEADS = 32
BM = 256
CW = 512
PAD = 48
EPS = 1e-5
F32, BF16, U32 = jnp.float32, jnp.bfloat16, jnp.uint32

PV_DELAY, PV_DELAY_FIRST = 10, 14
PROJ_ORDER = (4, 0, 2, 5, 1, 3)
O_STEPS, PREP_EARLY, PREP_LATE = 97, 0.2, 0.05
HEAD_MM, HEAD_ATT, TAIL_ATT, TAIL_MM, LAST_MM = 21, 8, 10, 39, 85
HEAD_START, GELU_STEPS, FIRST_ROWS = 7, 5, 32


def _merge(*streams):
    def gen():
        state = [[g, max(n, 1), 0] for g, n in streams]
        while state:
            s = min(state, key=lambda e: (e[2] + 0.5) / e[1])
            try:
                next(s[0])
                s[2] += 1
                yield
            except StopIteration:
                state.remove(s)
    return gen(), sum(n for _, n in streams)


def _chain(*streams):
    def gen():
        for g, _ in streams:
            yield from g
    return gen(), sum(n for _, n in streams)


def _cut(stream, *sizes):
    g, n = stream
    return [((next(g) for _ in range(k)), k) for k in sizes] + [(g, n - sum(sizes))]


def _run(*streams):
    for _ in _merge(*streams)[0]:
        pass


def _cat(xs, axis):
    return xs[0] if len(xs) == 1 else jnp.concatenate(xs, axis=axis)


class _Slabs:
    def __init__(self, ref, rows, base=0):
        self.ref, self.rows, self.base, self.step = ref, rows, base, rows + PAD

    def window(self, first, count):
        start = self.base + first * self.step
        if isinstance(start, int):
            return _Slabs(self.ref, self.rows, start)
        return _Slabs(self.ref.at[pl.ds(pl.multiple_of(start, 16), count * self.step)], self.rows)

    def slab(self, idx):
        return self.ref.at[pl.ds(self.base + idx * self.step, self.rows)]

    def words(self, idx, r0=0, r1=None):
        start = self.base + idx * self.step
        return self.ref.bitcast(U32)[(start + r0) // 2:(start + (r1 or self.rows)) // 2, :]

    def load(self, idx, r0=0, r1=None):
        return pltpu.bitcast(self.words(idx, r0, r1), BF16)

    def store(self, idx, r0, v):
        start = self.base + idx * self.step + r0
        self.ref[start:start + v.shape[0], :] = v.astype(BF16)


class _Order:
    def __init__(self, never, every):
        self.never, self.every, self.latest, self.pending = never, every, None, []

    def _tie(self, dep, v):
        head = jnp.where(self.never, dep, v[0:8, 0:128])
        head = _cat([head] + ([v[0:8, 128:]] if v.shape[1] > 128 else []), 1)
        return _cat([head] + ([v[8:]] if v.shape[0] > 8 else []), 0)

    def after_matmul(self, v):
        return self._tie(self.latest, v)

    def before_matmul(self, v):
        self.pending.append(v[0:8, 0:128])

    def matmul(self, lhs_words, rhs):
        for dep in self.pending:
            lhs_words = self._tie(pltpu.bitcast(dep, U32), lhs_words)
        self.pending = []
        r = jnp.dot(pltpu.bitcast(lhs_words, BF16), rhs, preferred_element_type=F32)
        self.latest = r[0:8, 0:128]
        return r


_FLIP = (1, 0, 1, 1, 0, 0, 1)


def _add(p, q, sign=1):
    if isinstance(p, list):
        return [_add(a, b, sign) for a, b in zip(p, q)]
    return p + q if sign > 0 else p - q


def _operands(g, left, flip=0):
    n = len(g) // 2
    x11, x12 = [r[:n] for r in g[:n]], [r[n:] for r in g[:n]]
    x21, x22 = [r[:n] for r in g[n:]], [r[n:] for r in g[n:]]
    if left:
        terms = [(x21, x11, -1), (x11, x22), (x12, x22, -1), (x21, x22), (x22,), (x11,), (x11, x12)]
    else:
        if flip:
            x11, x12, x21, x22 = x12, x11, x22, x21
        terms = [(x11, x12), (x11, x22), (x21, x22), (x11,), (x21, x11, -1), (x12, x22, -1), (x22,)]
    for t in terms:
        yield t[0] if len(t) == 1 else _add(*t)


def _combine(sub, flip=0):
    m6 = yield from sub(0)
    m1 = yield from sub(1)
    c22 = _add(m6, m1)
    m7 = yield from sub(2)
    c11 = _add(m1, m7)
    m2 = yield from sub(3)
    c22 = _add(c22, m2, -1)
    m4 = yield from sub(4)
    c11 = _add(c11, m4)
    c21 = _add(m2, m4)
    m3 = yield from sub(5)
    c22 = _add(c22, m3)
    m5 = yield from sub(6)
    c11 = _add(c11, m5, -1)
    c12 = _add(m3, m5)
    if flip:
        c11, c12, c21, c22 = c12, c11, c22, c21
    return [a + b for a, b in zip(c11, c12)] + [a + b for a, b in zip(c21, c22)]


def _split(load, rows, cols, left, dst, stride, order=None, load_steps=0, groups=None):
    br, bc = rows // 4, cols // 4
    groups = range(0, br, 16) if groups is None else groups

    def gen():
        for r0 in groups:
            for t in range(bc // 128):
                g = []
                for a in range(4):
                    g.append([load(a * br + r0, b * bc + t * 128) for b in range(4)])
                    for _ in range(load_steps):
                        yield
                for i, half in enumerate(_operands(g, left)):
                    for k, ((v,),) in enumerate(_operands(half, left, _FLIP[i])):
                        dst.store((7 * i + k) * stride + t, r0, v)
                        if order is not None and (7 * i + k) % order.every == 1:
                            order.before_matmul(v)
                    yield
    return gen(), len(groups) * bc // 128 * (7 + 4 * load_steps)


def _strassen(product, finish):
    def leaf(p):
        r = product(p)
        yield
        return [[r]]

    def gen():
        grid = yield from _combine(lambda i: _combine(lambda k: leaf(7 * i + k), _FLIP[i]))
        br, bc = grid[0][0].shape
        finish({(a * br, b * bc + t): blk[:, t:t + 128]
                for a, row in enumerate(grid) for b, blk in enumerate(row) for t in range(0, bc, 128)})
    return gen(), 49


def _project(lhs, rhs, order, finish):
    return _strassen(
        lambda p: order.matmul(_cat([lhs.words(2 * p), lhs.words(2 * p + 1)], 1), rhs.load(p)), finish)


def _gelu(x):
    c0 = float(np.sqrt(2.0 / np.pi))
    hx = 0.5 * x
    return hx + hx * jnp.tanh(x * (c0 + (c0 * 0.044715) * (x * x)))


def _lane_block(rows):
    return lax.broadcasted_iota(jnp.int32, (rows, 128), 1) >> 5


def _butterfly(a):
    blk = _lane_block(next(v for v in a if v is not None).shape[0])

    def pick(bit, p, q):
        if p is None and q is None:
            return None
        zero = jnp.zeros_like(q if p is None else p)
        return jnp.where((blk & bit) == 0, zero if p is None else p, zero if q is None else q)
    b = [pick(1, a[h], a[h ^ 1]) for h in range(4)]
    return [pick(2, b[h], b[h ^ 2]) for h in range(4)]


def _attention(qt, k_prev, k_cur, vt_prev, vt_cur, p_s, o_s, delay):
    groups = o_s.shape[1] // 128
    units = [(j, g) for g in range(groups) for j in range(BM // 128)]
    if k_prev is None:
        units.sort(reverse=True)
    stats = [[] for _ in units]
    tri = (lax.broadcasted_iota(jnp.int32, (32, 128), 0)
           > (lax.broadcasted_iota(jnp.int32, (32, 128), 1) & 31))
    pair = 2 * lax.broadcasted_iota(jnp.int32, (16, 128), 0)
    col = lax.broadcasted_iota(jnp.int32, (16, 128), 1) & 31
    tri_words = pltpu.bitcast(jnp.where(pair > col, 0xFFFF, 0) | jnp.where(pair + 1 > col, -0x10000, 0), U32)
    dot = lambda a, b: jnp.dot(pltpu.bitcast(a, BF16), pltpu.bitcast(b, BF16), preferred_element_type=F32)

    def lowest(j, t):
        return max(t, 8 - 4 * j) if k_prev is None else t

    def keys(g, r):
        return k_prev.words(g, r, r + 32) if r < BM else k_cur.words(g, r - BM, r - BM + 32)

    def scores(u):
        j, g = units[u]
        for t in range(4):
            q = [qt.words(j * groups + g, 32 * h, 32 * h + 32) for h in range(4)]
            qd = _cat([jnp.where(_lane_block(16) == (h ^ t), q[h], jnp.zeros_like(q[h])) for h in range(4)], 0)
            lo = lowest(j, t)
            outer = [a for a in range(lo, t + 9) if not 4 <= a < 8]
            for part, blocks in enumerate((outer, list(range(max(lo, 4), 8)))):
                if blocks:
                    k = _cat([keys(g, j * 128 + 32 * a) for a in blocks], 0)
                    step = k.shape[0] // min(len(blocks), 2)
                    s = _cat([dot(k[r:r + step], qd) for r in range(0, k.shape[0], step)], 0)
                    s = [s[r:r + 32] for r in range(0, s.shape[0], 32)]
                    if part == 0 and lo == t:
                        s = s[1:-1] + [jnp.where(tri, s[0], s[-1])]
                    elif part == 0:
                        s[-1] = jnp.where(tri, -jnp.inf, s[-1])
                    m = jnp.max(functools.reduce(jnp.maximum, s), axis=0, keepdims=True)
                    e = [jnp.exp2(b - m) for b in s]
                    stats[u].append((part, m, jnp.sum(functools.reduce(jnp.add, e), axis=0, keepdims=True)))
                    for a, b in zip(blocks[len(blocks) - len(e):], e):
                        p_s.store(u % 3 * 4 + t, (a - t) * 32, b)
                yield

    def by_head(u, part, which):
        v = [jnp.broadcast_to(s[which], (8, 128)) for s in stats[u] if s[0] == part]
        t = lax.broadcasted_iota(jnp.int32, (8, 128), 0) ^ _lane_block(8)
        return jnp.where((t & 2) == 0, jnp.where((t & 1) == 0, v[0], v[1]), jnp.where((t & 1) == 0, v[2], v[3]))

    def values(u):
        j, g = units[u]
        outer, middle = [None] * 4, [None] * 4
        for tile in range(3):
            if lowest(j, 0) >= 4 * tile + 4:
                yield
                yield
                continue
            p = []
            for a in range(4 * tile, 4 * tile + 4):
                src = [None] * 4
                for t in range(4):
                    if lowest(j, t) <= a <= t + 8:
                        r = (8 if a == t else a - t) * 32
                        src[t] = p_s.words(u % 3 * 4 + t, r, r + 32)
                        if a == t or (a == t + 8 and lowest(j, t) == t):
                            src[t] = src[t] & (tri_words if a == t else ~tri_words)
                p.append(_butterfly(src))
            yield
            vt, acc = vt_prev if j + tile < 2 else vt_cur, middle if tile == 1 else outer
            for h in range(4):
                r = dot(vt.words((j + tile) % 2 * groups + g, 32 * h, 32 * h + 32), _cat([b[h] for b in p], 0))
                acc[h] = r if acc[h] is None else acc[h] + r
            yield
        row = lambda v, h: jnp.broadcast_to(v[h:h + 1], (32, 128))
        m0, l0 = by_head(u, 0, 1), by_head(u, 0, 2)
        if middle[0] is None:
            c0 = 1.0 / l0
            ot = [outer[h] * row(c0, h) for h in range(4)]
        else:
            m1, l1 = by_head(u, 1, 1), by_head(u, 1, 2)
            m = jnp.maximum(m0, m1)
            c0, c1 = jnp.exp2(m0 - m), jnp.exp2(m1 - m)
            inv = 1.0 / (c0 * l0 + c1 * l1)
            c0, c1 = c0 * inv, c1 * inv
            ot = [outer[h] * row(c0, h) + middle[h] * row(c1, h) for h in range(4)]
        o = _cat(ot, 0).T
        yield
        for t, v in enumerate(_butterfly([o[r:r + 32] for r in range(0, 128, 32)])):
            o_s[j * 128 + 32 * t:j * 128 + 32 * t + 32, g * 128:(g + 1) * 128] = v
        yield

    def gen():
        first = (None for u in range(len(units)) for _ in scores(u))
        second = (None for u in range(len(units)) for _ in values(u))
        for step in range(8 * len(units) + delay):
            next(first, None)
            if step >= delay:
                next(second, None)
            yield
    return gen(), 8 * len(units) + delay


def _slab_buffers(d, f):
    n = d // 128
    return dict(
        raw=(4 * n, d),
        wa=(49 * 4 * d // CW, d // 4), w1=(49 * f // CW, d // 4), w2=(49 * 2, f // 4),
        y=(49 * 2, BM // 4), o=(49 * 2, BM // 4), z=(49 * 2, BM // 4), g=(49 * f // CW, BM // 4),
        qt=(2 * n, 128), k=(2 * n, BM), vt=(4 * n, 128), p=(12, 288))


def _kernel(x_hbm, wqkv_hbm, wo_hbm, w1_hbm, b1_hbm, w2_hbm, b2_hbm, out_hbm,
            h_s, o_s, b1_raw, b2_raw, b1_s, b2_s, x_next, x_prev, raw1, raw2, out_s,
            b_sem, x_sem, raw_sem, w_sem, out_sem, fence_sem, step_s, *pools):
    seq, d = x_hbm.shape
    f = w1_hbm.shape[1]
    nb, ng, nc = seq // BM, d // 128, f // CW
    scale = float((d // HEADS) ** -0.5 * np.log2(np.e))
    raw, wa, w1, w2, y, o, z, g, qt, k, vt, p_s = [
        _Slabs(ref, rows) for ref, (_, rows) in zip(pools, _slab_buffers(d, f).values())]

    block = lambda ref, b: ref.at[pl.ds(pl.multiple_of(b * BM, BM), BM)]
    next_copy = lambda b: pltpu.make_async_copy(block(x_hbm, b), x_next, x_sem.at[0])
    prev_copy = lambda b: pltpu.make_async_copy(block(x_hbm, b), x_prev, x_sem.at[1])
    out_copy = lambda b: pltpu.make_async_copy(out_s.at[b % 2], block(out_hbm, b), out_sem.at[b % 2])
    mlp_copies = lambda c: [
        pltpu.make_async_copy(w1_hbm.at[:, pl.ds(c * CW, CW)], raw1.at[c % 2], w_sem.at[c % 2]),
        pltpu.make_async_copy(w2_hbm.at[pl.ds(c * CW, CW)], raw2.at[c % 2], w_sem.at[2 + c % 2])]

    def raw_copies(c, tiles=range(4)):
        src, col = (wo_hbm, (c - 6) * CW) if isinstance(c, int) and c >= 6 else (wqkv_hbm, c * CW)
        dst = raw.window(c * 4, 4)
        return [pltpu.make_async_copy(src.at[:, pl.ds(pl.multiple_of(col + t * 128, 128), 128)],
                                      dst.slab(t), raw_sem.at[c]) for t in tiles]

    def start(copies):
        for cp in copies:
            cp.start()

    def wait(copies):
        for cp in copies:
            cp.wait()

    def fence():
        pl.semaphore_signal(fence_sem, 1)
        pl.semaphore_wait(fence_sem, 1)

    def pieces(ref):
        return lambda r0, c0: ref[r0:r0 + 16, c0:c0 + 128].astype(F32)

    def split_chunk(c, order=None):
        src = raw.window(c * 4, 4)
        return _split(lambda r0, c0: src.slab(c0 // 128)[r0:r0 + 16, :].astype(F32),
                      d, CW, False, wa.window(c * 49, 49), 1, order)

    def normalized(rows, times, dst, order, groups=range(0, BM // 4, 16)):
        done = {}

        def layer_norm(r):
            for r0 in range(r, BM, BM // 4):
                v = rows[r0:r0 + 16, :].astype(F32)
                for _ in range(times):
                    mean = jnp.mean(v, axis=-1, keepdims=True)
                    order.before_matmul(jnp.broadcast_to(mean, (16, 128)))
                    yield
                    v = v - mean
                    v = v * lax.rsqrt(jnp.mean(v * v, axis=-1, keepdims=True) + EPS)
                    order.before_matmul(v)
                    yield
                done[r0] = v
        return _chain(*[s for r in groups for s in (
            (layer_norm(r), 8 * times),
            _split(lambda r0, c0: done[r0][:, c0:c0 + 128], BM, d, True, dst, 2, order, 0, [r]))])

    def store_queries(idx, v):
        v = _cat(_butterfly([v[r:r + 32] for r in range(0, 128, 32)]), 0).T
        qt.store(idx, 0, v)
        return v

    def out_proj(b, order):
        h_rows = block(h_s, b)

        def finish(c, tiles):
            for (r0, c0), v in tiles.items():
                at = slice(r0, r0 + v.shape[0]), slice(c * CW + c0, c * CW + c0 + 128)
                h_rows[at] = x_prev[at].astype(F32) + v
        return _chain(*[_project(o, wa.window((6 + c) * 49, 49), order, functools.partial(finish, c))
                        for c in range(2)])

    biases = [pltpu.make_async_copy(b1_hbm, b1_raw, b_sem.at[0]), pltpu.make_async_copy(b2_hbm, b2_raw, b_sem.at[1])]
    start(biases + [prev_copy(0)])
    wait(biases)
    start(raw_copies(0))
    b1_s[...] = jnp.broadcast_to(b1_raw[...].astype(F32).reshape(1, f), (8, f))
    b2_s[...] = jnp.broadcast_to(b2_raw[...].astype(F32).reshape(1, d), (8, d))
    wait([prev_copy(0)])
    y0, x0 = _Slabs(z.ref, BM), x_prev[...].astype(F32)
    x0 = x0 - jnp.mean(x0, axis=-1, keepdims=True)
    x0 = x0 * lax.rsqrt(jnp.mean(x0 * x0, axis=-1, keepdims=True) + EPS)
    for t in range(ng):
        y0.store(t, 0, x0[:, t * 128:(t + 1) * 128])
    start(raw_copies(1, (0, 1)))

    def plain_proj(c, store, order):
        src = raw.window(c * 4, 4)

        def gen():
            for t in range(4):
                for r0 in range(0, BM, FIRST_ROWS):
                    lhs = _cat([y0.words(a, r0, r0 + FIRST_ROWS) for a in range(ng)], 1)
                    store(t, r0, order.matmul(lhs, src.load(t)))
                    yield
        return gen(), 4 * BM // FIRST_ROWS

    @pl.loop(0, 4)
    def _(c):
        order, step_s[0] = _Order(c < 0, 7), c
        wait(raw_copies(c))
        start(raw_copies(c + 1, (2, 3)) + raw_copies(c + 2, (0, 1)))
        pl.when(c == 2)(lambda: start([next_copy(1)]))
        pl.when(c == 3)(lambda: start(raw_copies(5, (2, 3)) + raw_copies(6, (0, 1, 2))))
        fence()
        mul, dst = jnp.where(c < 2, scale, 1.0), k.window((c * 4 + ng) % (2 * ng), 4)
        _run(plain_proj(c, lambda t, r0, r: dst.store(t, r0, r * mul), order), split_chunk(c, order))

    wait([next_copy(1)])
    for c in range(2):
        order, rows = _Order(step_s[0] < 0, 7), []
        wait(raw_copies(4 + c))
        start(raw_copies(6, (3,)) + raw_copies(7) if c == 0 else [])
        fence()

        def store_values(t, r0, r):
            rows.append(r)
            if (r0 + FIRST_ROWS) % 128 == 0:
                vt.store(r0 // 128 * ng + c * 4 + t, 0, _cat(rows[-128 // FIRST_ROWS:], 0).T)

        def queries():
            for t in range(c * 4, c * 4 + 4):
                for j in range(2):
                    v = k.slab(ng + t)[j * 128:(j + 1) * 128, :].astype(F32)
                    order.before_matmul(store_queries(j * ng + t, v))
                    yield
        _run(plain_proj(4 + c, store_values, order),
             _chain(split_chunk(4 + c, order), normalized(x_next, 1, y, order, [c * 32, c * 32 + 16])),
             (queries(), 8))

    wait(raw_copies(6) + raw_copies(7))
    start(mlp_copies(0))
    fence()
    _run(_attention(qt, None, k, None, vt, p_s, o_s, PV_DELAY_FIRST), _chain(split_chunk(6), split_chunk(7)))

    @pl.loop(1, nb)
    def _(i):
        order, step_s[0], c = _Order(i < 0, 9), i, i - 1
        rows = [next_copy(jnp.minimum(i + 1, nb - 1)), prev_copy(c)]
        wait(mlp_copies(c))
        start(rows)
        pl.when(i < nc)(lambda: start(mlp_copies(i)))
        fence()
        w2_rows = w2.ref.at[pl.ds(pl.multiple_of(c * 128, 128), w2.ref.shape[0] - (nc - 1) * 128)]
        prep = _chain(_split(pieces(raw1.at[c % 2]), d, CW, False, w1.window(c * 49, 49), 1, order),
                      _split(pieces(raw2.at[c % 2]), CW, d, False, _Slabs(w2_rows, w2.rows), 2, order))
        k_new, vt_new = k.window(i % 2 * ng, ng), vt.window(i % 2 * 2 * ng, 2 * ng)

        def finish(chunk, tiles):
            for t in range(4):
                v, a = _cat([tiles[at] for at in sorted(tiles) if at[1] == t * 128], 0), chunk % 2 * 4 + t
                for j in range(2):
                    part = v[j * 128:(j + 1) * 128]
                    if chunk < 2:
                        store_queries(j * ng + a, part * scale)
                    elif chunk < 4:
                        k_new.store(a, j * 128, part)
                    else:
                        vt_new.store(j * ng + a, 0, part.T)
        proj = _chain(*[_project(y, wa.window(n * 49, 49), order, functools.partial(finish, n)) for n in PROJ_ORDER])
        proj = _cut(proj, O_STEPS, proj[1] - O_STEPS - HEAD_MM)
        early, late = int(prep[1] * PREP_EARLY), int(prep[1] * PREP_LATE)
        prep = _cut(prep, early, prep[1] - early - late)
        _run(proj[0], _chain(_split(pieces(o_s), BM, d, True, o, 2, order), prep[0]))
        _run(proj[1], prep[1])
        wait(rows)
        fence()
        att = _attention(
            qt.window(jnp.minimum(i, 0), 2 * ng), k.window((i + 1) % 2 * ng, ng), k.window((i & 1) * ng, ng),
            vt.window((i + 1) % 2 * 2 * ng, 2 * ng), vt.window((i & 1) * 2 * ng, 2 * ng), p_s, o_s, PV_DELAY)
        att = _cut(att, HEAD_ATT, att[1] - HEAD_ATT - TAIL_ATT)
        _run(proj[2], att[0])
        _run(att[1])
        fence()
        wo = _cut(out_proj(c, order), TAIL_MM)
        _run(att[2], wo[0])
        _run(wo[1], _chain(normalized(x_next, 1, y, order), prep[2]))

    order = _Order(step_s[0] < 0, 7)
    start([prev_copy(nb - 1)])
    fence()
    _run(_split(pieces(o_s), BM, d, True, o, 2))
    wait([prev_copy(nb - 1)])
    wo = _cut(out_proj(nb - 1, order), LAST_MM)
    _run(wo[0], normalized(block(h_s, 0), 2, z, order))
    _run(wo[1])

    @pl.loop(0, nb)
    def _(i):
        order, hidden, early = _Order(i < 0, 11), {}, {}
        pl.when(i >= 2)(lambda: wait([out_copy(i - 2)]))
        up = lambda c: _project(z, w1.window(c * 49, 49), order, lambda tiles: hidden.update({c: tiles}))

        def activate(c):
            def load(r0, c0):
                bias = order.after_matmul(b1_s[:, c * CW + c0:c * CW + c0 + 128])
                return _gelu(hidden[c][(r0 // 64 * 64, c0)][r0 % 64:r0 % 64 + 16] + _cat([bias, bias], 0))
            return _split(load, BM, CW, True, g.window(c, 1), nc, None, GELU_STEPS)

        def down(p, c0, c1):
            return order.matmul(_cat([g.words(p * nc + c) for c in range(c0, c1)], 1),
                                _cat([w2.load(p * 2 + t, c0 * 128, c1 * 128) for t in range(2)], 1))

        def head_start():
            for p in range(HEAD_START):
                early[p] = down(p, 0, nc - 1)
                yield

        def finish(tiles):
            h_rows, dst = block(h_s, i), out_s.at[i % 2]
            for (r0, c0), v in tiles.items():
                at = slice(r0, r0 + v.shape[0]), slice(c0, c0 + 128)
                dst[at] = (h_rows[at] + (v + _cat([b2_s[:, c0:c0 + 128]] * 8, 0))).astype(dst.dtype)

        _run(up(0))
        for c in range(1, nc):
            _run(up(c), activate(c - 1))
        _run((head_start(), HEAD_START), activate(nc - 1))
        _run(_strassen(lambda p: early[p] + down(p, nc - 1, nc) if p in early else down(p, 0, nc), finish),
             normalized(block(h_s, jnp.minimum(i + 1, nb - 1)), 2, z, order))
        start([out_copy(i)])

    wait([out_copy(nb - 2), out_copy(nb - 1)])


@jax.jit
def pallas_sequential_preLN__sliding_block__mixer_channel_mlp__prompt_kernel(
    A_x: jax.Array,
    A_wqkv: jax.Array,
    A_wo: jax.Array,
    B_x: jax.Array,
    B_w1: jax.Array,
    B_b1: jax.Array,
    B_w2: jax.Array,
    B_b2: jax.Array,
):
    batch, seq, d = A_x.shape
    f = B_w1.shape[1]
    assert (batch, d) == (1, 2 * CW) and seq // BM == f // CW + 1
    vmem, dma = pltpu.VMEM, pltpu.SemaphoreType.DMA
    out = pl.pallas_call(
        _kernel,
        in_specs=[pl.BlockSpec(memory_space=pl.ANY)] * 7,
        out_specs=pl.BlockSpec(memory_space=pl.ANY),
        out_shape=jax.ShapeDtypeStruct((seq, d), A_x.dtype),
        scratch_shapes=[
            vmem((seq, d), F32), vmem((BM, d), F32),
            vmem((f,), B_b1.dtype), vmem((d,), B_b2.dtype), vmem((8, f), F32), vmem((8, d), F32),
            vmem((BM, d), A_x.dtype), vmem((BM, d), A_x.dtype),
            vmem((2, d, CW), B_w1.dtype), vmem((2, CW, d), B_w2.dtype), vmem((2, BM, d), A_x.dtype),
            dma((2,)), dma((2,)), dma((8,)), dma((4,)), dma((2,)), pltpu.SemaphoreType.REGULAR,
            pltpu.SMEM((1,), jnp.int32),
            *[vmem((n * (rows + PAD), 128), BF16) for n, rows in _slab_buffers(d, f).values()]],
        compiler_params=pltpu.CompilerParams(vmem_limit_bytes=127 << 20, disable_bounds_checks=True),
        name="fused",
    )(A_x.reshape(seq, d), A_wqkv, A_wo, B_w1, B_b1, B_w2, B_b2)
    return out.reshape(batch, seq, d)
```
